```python
import os as _os
_os.environ.setdefault("JAX_PLATFORMS", "cpu")
import jax
import jax.numpy as jnp

def _softmax(x, axis=-1):
    return jax.nn.softmax(x, axis=axis)
def _gelu(x):
    return jax.nn.gelu(x, approximate=True)
def _silu(x):
    return jax.nn.silu(x)
def _sigmoid(x):
    return jax.nn.sigmoid(x)
def _layernorm(x, axis=-1, eps=1e-5):
    m = jnp.mean(x, axis=axis, keepdims=True)
    v = jnp.var(x, axis=axis, keepdims=True)
    return (x - m) / jnp.sqrt(v + eps)
def _scatter_add(tgt, idx, src, axis=0):
    return tgt.at[idx].add(src)
def _segment_sum(src, seg, n):
    return jax.ops.segment_sum(src, seg, n)
class _Rng:
    def __init__(self, key):
        self._k = key
    def _next(self):
        self._k, sub = jax.random.split(self._k)
        return sub
    def normal(self, shape):
        return jax.random.normal(self._next(), shape, dtype=jnp.bfloat16)
    def randint(self, lo, hi, shape):
        return jax.random.randint(self._next(), shape, lo, hi, dtype=jnp.int32)
    def uniform(self, shape, lo=0.0, hi=1.0):
        return jax.random.uniform(self._next(), shape, jnp.bfloat16, lo, hi)
    def permutation(self, n):
        return jax.random.permutation(self._next(), n)


kernel_name = 'sequential_preLN__softmax_full_mha__glu_gated_swiglu__prompt'

def setup_inputs():
    _rng = _Rng(jax.random.key(int.from_bytes(__import__("os").urandom(4), "little")))
    _w = (lambda a: (lambda t: t.astype(jnp.bfloat16) if jnp.issubdtype(t.dtype, jnp.floating) else t)(jnp.asarray(a)))
    def _A_setup():
        B, S, D = 1, 2048, 640
        return {
            "x": _w((lambda *s: _rng.normal(s) * 0.05)(B, S, D)),
            "wqkv": _w((lambda *s: _rng.normal(s) * 0.05)(D, 3 * D)),
            "wo": _w((lambda *s: _rng.normal(s) * 0.05)(D, D)),
        }
    _A_in = _A_setup()

    def _B_setup():
        B, S, D, F = 1, 2048, 640, 1728
        return {
            "x": _w((lambda *s: _rng.normal(s) * 0.05)(B, S, D)),
            "w1": _w((lambda *s: _rng.normal(s) * 0.05)(D, F) * (2.0 / D) ** 0.5),
            "w3": _w((lambda *s: _rng.normal(s) * 0.05)(D, F) * (2.0 / D) ** 0.5),
            "w2": _w((lambda *s: _rng.normal(s) * 0.05)(F, D) * (2.0 / F) ** 0.5),
        }
    _B_in = _B_setup()

    return {
        "A_x": _A_in["x"],
        "A_wqkv": _A_in["wqkv"],
        "A_wo": _A_in["wo"],
        "B_x": _B_in["x"],
        "B_w1": _B_in["w1"],
        "B_w3": _B_in["w3"],
        "B_w2": _B_in["w2"],
    }

def reference(A_x, A_wqkv, A_wo, B_x, B_w1, B_w3, B_w2):
    def _A_ref(x, wqkv, wo):
        B, S, D = x.shape
        H = 32; Dh = D // H
        qkv = (lambda x, *d: x.transpose(*d))((x @ wqkv).reshape(B, S, 3, H, Dh), 2, 0, 3, 1, 4)
        q, k, v = qkv[0], qkv[1], qkv[2]
        scale = Dh ** -0.5
        scores = jnp.einsum("bhqd,bhkd->bhqk", q, k) * scale
        p = _softmax(scores, axis=-1)
        o = jnp.einsum("bhqk,bhkd->bhqd", p, v)
        return (lambda x, *d: x.transpose(*d))(o, 0, 2, 1, 3).reshape(B, S, D) @ wo

    def _B_ref(x, w1, w3, w2):
        gate = jnp.einsum("bsd,df->bsf", x, w1)
        up = jnp.einsum("bsd,df->bsf", x, w3)
        h = _silu(gate) * up
        out = jnp.einsum("bsf,fd->bsd", h, w2)
        return out

    x = A_x
    h = x + _A_ref(_layernorm(x, axis=-1), A_wqkv, A_wo)
    h2 = h + _B_ref(_layernorm(h, axis=-1), B_w1, B_w3, B_w2)
    return h2
```

```python
import functools
import math

import jax
import jax.numpy as jnp
import numpy as np
from jax import lax
from jax.experimental import pallas as pl
from jax.experimental.pallas import tpu as pltpu

S = 2048
D = 640
H = 32
DH = 20
F = 1728
HPW = 6
NWIN = 6
WSTRIDE = HPW * DH
EPS = 1e-5
LOG2E = math.log2(math.e)
L_MIN = 2.0 ** -60
F_CHUNKS = ((0, 512), (512, 512), (1024, 512), (1536, 192))

NT = (((1,), (1,)), ((), ()))


def _layernorm(x):
    m = jnp.mean(x, axis=-1, keepdims=True)
    xc = x - m
    v = jnp.mean(xc * xc, axis=-1, keepdims=True)
    return xc * lax.rsqrt(v + EPS)


def _make_kernel(bq, bm):
    nrb = S // bm

    def kernel(x_ref, wqkv_ref, wo_ref, w1_ref, w3_ref, w2_ref, out_ref,
               wt_ref, qtw_ref, kw_ref, vt_ref, ot_ref, qn_ref):
        step = pl.program_id(0)

        @pl.when(step == 0)
        def _project():
            wt_ref[...] = wqkv_ref[...].astype(jnp.float32).T.astype(jnp.bfloat16)
            r = lax.broadcasted_iota(jnp.int32, (8 * NWIN, D), 0)
            f = lax.broadcasted_iota(jnp.int32, (8 * NWIN, D), 1)
            head = (r // 8) * HPW + (r % 8)
            sel = jnp.where(((r % 8) < HPW) & (f // DH == head), 1.0, 0.0).astype(jnp.bfloat16)
            wrow = lax.broadcasted_iota(jnp.int32, (128, bm), 0)

            def rb_body(rb, kmax):
                r0 = pl.multiple_of(rb * bm, bm)
                xh = _layernorm(x_ref[pl.ds(r0, bm), :].astype(jnp.float32)).astype(jnp.bfloat16)
                qkvt = lax.dot_general(wt_ref[...], xh, NT, preferred_element_type=jnp.float32)
                q = (qkvt[0:D] * (DH ** -0.5 * LOG2E)).astype(jnp.bfloat16).astype(jnp.float32)
                k = qkvt[D:2 * D].astype(jnp.bfloat16).astype(jnp.float32)
                v = qkvt[2 * D:3 * D]
                qn_ref[:, pl.ds(r0, bm)] = jnp.dot(sel, (q * q).astype(jnp.bfloat16), preferred_element_type=jnp.float32)
                kn = jnp.dot(sel, (k * k).astype(jnp.bfloat16), preferred_element_type=jnp.float32)
                zpad = jnp.zeros((128, bm), jnp.float32)
                qp = jnp.concatenate([q, zpad], axis=0)
                kp = jnp.concatenate([k, zpad], axis=0)
                for c in range(NWIN):
                    lo = c * WSTRIDE
                    qtw_ref[c, 0:WSTRIDE, pl.ds(r0, bm)] = qp[lo:lo + WSTRIDE]
                    kwin = jnp.where(wrow < WSTRIDE, kp[lo:lo + 128], 1.0)
                    kw_ref[c, pl.ds(r0, bm), :] = kwin.T.astype(jnp.bfloat16)
                ones = jnp.ones((8, bm), jnp.float32)
                for h in range(H):
                    a = (h * DH) // 8 * 8
                    vt_ref[h, :, pl.ds(r0, bm)] = jnp.concatenate([v[a:a + 24], ones], axis=0).astype(jnp.bfloat16)
                return jnp.maximum(kmax, kn)

            kmax = lax.fori_loop(0, nrb, rb_body, jnp.zeros((8 * NWIN, bm), jnp.float32))
            kmax = jnp.max(kmax, axis=1, keepdims=True)
            bound = jnp.sqrt(qn_ref[...] * kmax) * (1.0 + 2.0 ** -6)
            for c in range(NWIN):
                qtw_ref[c, WSTRIDE:128, :] = -bound[8 * c:8 * c + 8]

        q0 = pl.multiple_of(step * bq, bq)
        rows = lax.broadcasted_iota(jnp.int32, (128, bq), 0)
        row8 = lax.broadcasted_iota(jnp.int32, (8, bq), 0)

        def head_acc(h, use_true_max):
            c = h // HPW
            hl = h - c * HPW
            qw = qtw_ref[c, :, pl.ds(q0, bq)]
            mask = (rows >= hl * DH) & (rows < hl * DH + DH)
            if not use_true_max:
                mask = mask | (rows == WSTRIDE + hl)
            qm = jnp.where(mask, qw, 0.0).astype(jnp.bfloat16)
            s = jnp.dot(kw_ref[c], qm, preferred_element_type=jnp.float32)
            if use_true_max:
                s = s - jnp.max(s, axis=0, keepdims=True)
            p = jnp.exp2(s).astype(jnp.bfloat16)
            return jnp.dot(vt_ref[h], p, preferred_element_type=jnp.float32)

        def pair(p, use_true_max):
            ae = head_acc(2 * p, use_true_max)
            ao = head_acc(2 * p + 1, use_true_max)
            le, lo = ae[24:32], ao[24:32]
            re, ro = 1.0 / le, 1.0 / lo
            mid = jnp.where(row8 < 4, ae[16:24] * re, ao[0:8] * ro)
            blk = jnp.concatenate([ae[0:8] * re, ae[8:16] * re, mid, ao[8:16] * ro, ao[16:24] * ro], axis=0)
            ot_ref[pl.ds(pl.multiple_of(p * 2 * DH, 8), 2 * DH), :] = blk
            return jnp.minimum(le, lo)

        def fast_body(p, lmin):
            return jnp.minimum(lmin, pair(p, False))

        lmin = lax.fori_loop(0, H // 2, fast_body, jnp.ones((8, bq), jnp.float32))
        ok = jnp.min(jnp.where(lmin >= L_MIN, 1.0, 0.0))

        @pl.when(ok < 0.5)
        def _fallback():
            def slow_body(p, carry):
                pair(p, True)
                return carry
            lax.fori_loop(0, H // 2, slow_body, 0)

        o = ot_ref[...].T.astype(jnp.bfloat16)
        h = x_ref[pl.ds(q0, bq), :].astype(jnp.float32) + jnp.dot(o, wo_ref[...], preferred_element_type=jnp.float32)
        hn = _layernorm(h).astype(jnp.bfloat16)
        y = h
        for f0, fw in F_CHUNKS:
            g = jnp.dot(hn, w1_ref[:, f0:f0 + fw], preferred_element_type=jnp.float32)
            u = jnp.dot(hn, w3_ref[:, f0:f0 + fw], preferred_element_type=jnp.float32)
            a = (g * jax.nn.sigmoid(g) * u).astype(jnp.bfloat16)
            y = y + jnp.dot(a, w2_ref[f0:f0 + fw, :], preferred_element_type=jnp.float32)
        out_ref[...] = y.astype(out_ref.dtype)

    return kernel


@jax.jit
def pallas_sequential_preLN__softmax_full_mha__glu_gated_swiglu__prompt_kernel(
    A_x: jax.Array,
    A_wqkv: jax.Array,
    A_wo: jax.Array,
    B_x: jax.Array,
    B_w1: jax.Array,
    B_w3: jax.Array,
    B_w2: jax.Array,
):
    del B_x
    bq, bm = 512, 512
    x = A_x.reshape(S, D)
    full = lambda shape: pl.BlockSpec(shape, lambda i: (0,) * len(shape))
    out = pl.pallas_call(
        _make_kernel(bq, bm),
        grid=(S // bq,),
        in_specs=[full((S, D)), full((D, 3 * D)), full((D, D)), full((D, F)), full((D, F)), full((F, D))],
        out_specs=pl.BlockSpec((bq, D), lambda i: (i, 0)),
        out_shape=jax.ShapeDtypeStruct((S, D), A_x.dtype),
        scratch_shapes=[
            pltpu.VMEM((3 * D, D), jnp.bfloat16),
            pltpu.VMEM((NWIN, 128, S), jnp.float32),
            pltpu.VMEM((NWIN, S, 128), jnp.bfloat16),
            pltpu.VMEM((H, 32, S), jnp.bfloat16),
            pltpu.VMEM((D, bq), jnp.float32),
            pltpu.VMEM((8 * NWIN, S), jnp.float32),
        ],
        compiler_params=pltpu.CompilerParams(
            dimension_semantics=("arbitrary",), vmem_limit_bytes=110 * 1024 * 1024),
    )(x, A_wqkv, A_wo, B_w1, B_w3, B_w2)
    return out.reshape(A_x.shape)
```

```python
import functools
import math

import jax
import jax.numpy as jnp
import numpy as np
from jax import lax
from jax.experimental import pallas as pl
from jax.experimental.pallas import tpu as pltpu

S = 2048
D = 640
H = 32
DH = 20
F = 1728
HPW = 6
NWIN = 6
WSTRIDE = HPW * DH
EPS = 1e-5
LOG2E = math.log2(math.e)
L_MIN = 2.0 ** -60
L_MAX = 2.0 ** 12
FP = 1792
F_CHUNKS = ((0, 512), (512, 512), (1024, 512), (1536, 192))

NT = (((1,), (1,)), ((), ()))


def _layernorm(x, axis):
    m = jnp.mean(x, axis=axis, keepdims=True)
    xc = x - m
    v = jnp.mean(xc * xc, axis=axis, keepdims=True)
    return xc * lax.rsqrt(v + EPS)


def _make_kernel(bm, bt, sq, fch, wt_where):
    nrb = S // bm

    def kernel(x_hbm, wqkv_hbm, wo_hbm, w1t_hbm, w3t_hbm, w2_hbm, out_ref,
               x_ref, wqkv_ref, wo_ref, w1t_ref, w3t_ref, w2_ref,
               wt_ref, xt_ref, wot_ref, w2t_ref, qtw_ref, kw_ref, vt_ref, ot_ref, qn_ref, xsem, sems):
        step = pl.program_id(0)

        def head_acc(h, q0, nq, use_true_max):
            rows = lax.broadcasted_iota(jnp.int32, (128, nq), 0)
            c = h // HPW
            hl = h - c * HPW
            qw = qtw_ref[c, :, pl.ds(q0, nq)]
            mask = (rows >= hl * DH) & (rows < hl * DH + DH)
            if not use_true_max:
                mask = mask | (rows == WSTRIDE + hl)
            qm = jnp.where(mask, qw, 0.0).astype(jnp.bfloat16)
            s = jnp.dot(kw_ref[c], qm, preferred_element_type=jnp.float32)
            if use_true_max:
                s = s - jnp.max(s, axis=0, keepdims=True)
            p = jnp.exp2(s).astype(jnp.bfloat16)
            return jnp.dot(vt_ref[h], p, preferred_element_type=jnp.float32)

        def pair(p, q0, nq, use_true_max):
            row8 = lax.broadcasted_iota(jnp.int32, (8, nq), 0)
            ae = head_acc(2 * p, q0, nq, use_true_max)
            ao = head_acc(2 * p + 1, q0, nq, use_true_max)
            le, lo = ae[24:32], ao[24:32]
            re, ro = 1.0 / le, 1.0 / lo
            mid = jnp.where(row8 < 4, ae[16:24] * re, ao[0:8] * ro)
            blk = jnp.concatenate([ae[0:8] * re, ae[8:16] * re, mid, ao[8:16] * ro, ao[16:24] * ro], axis=0)
            ot_ref[pl.ds(pl.multiple_of(p * 2 * DH, 8), 2 * DH), pl.ds(q0, nq)] = blk
            return jnp.minimum(le, lo), jnp.maximum(le, lo)

        def x_copy(i):
            return pltpu.make_async_copy(x_hbm.at[pl.ds(i * bm, bm)], x_ref.at[pl.ds(i * bm, bm)], xsem.at[i])

        @pl.when(step == 0)
        def _project_and_attend():
            wcopy = pltpu.make_async_copy(wqkv_hbm, wqkv_ref, sems.at[0])
            ocopies = [
                pltpu.make_async_copy(wo_hbm, wo_ref, sems.at[1]),
                pltpu.make_async_copy(w2_hbm, w2_ref.at[pl.ds(0, F)], sems.at[2]),
                pltpu.make_async_copy(w1t_hbm, w1t_ref, sems.at[3]),
                pltpu.make_async_copy(w3t_hbm, w3t_ref, sems.at[4]),
            ]
            wcopy.start()
            x_copy(0).start()
            wcopy.wait()
            for i in range(1, nrb):
                x_copy(i).start()
            for cp in ocopies:
                cp.start()
            w2_ref[F:FP, :] = jnp.zeros((FP - F, D), jnp.bfloat16)
            wt_ref[...] = wqkv_ref[...].astype(jnp.float32).T.astype(jnp.bfloat16)

            r = lax.broadcasted_iota(jnp.int32, (8 * NWIN, D), 0)
            f = lax.broadcasted_iota(jnp.int32, (8 * NWIN, D), 1)
            head = (r // 8) * HPW + (r % 8)
            sel = jnp.where(((r % 8) < HPW) & (f // DH == head), 1.0, 0.0).astype(jnp.bfloat16)
            wrow = lax.broadcasted_iota(jnp.int32, (128, bm), 0)

            def rb_body(rb, kmax):
                r0 = pl.multiple_of(rb * bm, bm)
                x_copy(rb).wait()
                xb = x_ref[pl.ds(r0, bm), :]
                xt_ref[:, pl.ds(r0, bm)] = xb.T
                xh = _layernorm(xb.astype(jnp.float32), -1).astype(jnp.bfloat16)
                qkvt = lax.dot_general(wt_ref[...], xh, NT, preferred_element_type=jnp.float32)
                q = (qkvt[0:D] * (DH ** -0.5 * LOG2E)).astype(jnp.bfloat16).astype(jnp.float32)
                k = qkvt[D:2 * D].astype(jnp.bfloat16).astype(jnp.float32)
                v = qkvt[2 * D:3 * D]
                qn_ref[:, pl.ds(r0, bm)] = jnp.dot(sel, (q * q).astype(jnp.bfloat16), preferred_element_type=jnp.float32)
                kn = jnp.dot(sel, (k * k).astype(jnp.bfloat16), preferred_element_type=jnp.float32)
                zpad = jnp.zeros((128, bm), jnp.float32)
                qp = jnp.concatenate([q, zpad], axis=0)
                kp = jnp.concatenate([k, zpad], axis=0)
                for c in range(NWIN):
                    lo = c * WSTRIDE
                    qtw_ref[c, 0:WSTRIDE, pl.ds(r0, bm)] = qp[lo:lo + WSTRIDE]
                    kwin = jnp.where(wrow < WSTRIDE, kp[lo:lo + 128], 1.0)
                    kw_ref[c, pl.ds(r0, bm), :] = kwin.T.astype(jnp.bfloat16)
                ones = jnp.ones((8, bm), jnp.float32)
                for h in range(H):
                    a = (h * DH) // 8 * 8
                    vt_ref[h, :, pl.ds(r0, bm)] = jnp.concatenate([v[a:a + 24], ones], axis=0).astype(jnp.bfloat16)
                return jnp.maximum(kmax, kn)

            kmax = lax.fori_loop(0, nrb, rb_body, jnp.zeros((8 * NWIN, bm), jnp.float32))
            kmax = jnp.max(kmax, axis=1, keepdims=True)
            bound = jnp.sqrt(qn_ref[...] * kmax) * (1.0 + 2.0 ** -6)
            for c in range(NWIN):
                qtw_ref[c, WSTRIDE:128, :] = -bound[8 * c:8 * c + 8]

            for cp in ocopies:
                cp.wait()
            if wt_where == "pre":
                wot_ref[...] = wo_ref[...].T
                w2t_ref[...] = w2_ref[...].T

            def fast_body(p, carry):
                lmin, lmax = pair(p, 0, S, False)
                if wt_where == "loop":
                    f0 = pl.multiple_of(jnp.minimum(p, FP // 128 - 1) * 128, 128)
                    w2t_ref[:, pl.ds(f0, 128)] = w2_ref[pl.ds(f0, 128), :].T
                    o0 = pl.multiple_of(jnp.minimum(p, 4) * 128, 128)
                    wot_ref[:, pl.ds(o0, 128)] = wo_ref[pl.ds(o0, 128), :].T
                return jnp.minimum(carry[0], lmin), jnp.maximum(carry[1], lmax)

            ones8 = jnp.ones((8, S), jnp.float32)
            lmin, lmax = lax.fori_loop(0, H // 2, fast_body, (ones8, ones8))
            ok = jnp.min(jnp.where((lmin >= L_MIN) & (lmax <= L_MAX), 1.0, 0.0))

            @pl.when(ok < 0.5)
            def _fallback():
                def slow_body(i, carry):
                    qb = i // (H // 2)
                    p = i - qb * (H // 2)
                    pair(p, pl.multiple_of(qb * sq, sq), sq, True)
                    return carry
                lax.fori_loop(0, (S // sq) * (H // 2), slow_body, 0)

        q0 = pl.multiple_of(step * bt, bt)
        o = ot_ref[:, pl.ds(q0, bt)].astype(jnp.bfloat16)
        h = xt_ref[:, pl.ds(q0, bt)].astype(jnp.float32) + jnp.dot(wot_ref[...], o, preferred_element_type=jnp.float32)
        hn = _layernorm(h, 0).astype(jnp.bfloat16)
        y = h
        for f0, fw in fch:
            g = jnp.dot(w1t_ref[f0:f0 + fw, :], hn, preferred_element_type=jnp.float32)
            u = jnp.dot(w3t_ref[f0:f0 + fw, :], hn, preferred_element_type=jnp.float32)
            a = (g * jax.nn.sigmoid(g) * u).astype(jnp.bfloat16)
            y = y + jnp.dot(w2t_ref[:, f0:f0 + fw], a, preferred_element_type=jnp.float32)
        out_ref[...] = y.astype(out_ref.dtype).T

    return kernel


@jax.jit
def pallas_sequential_preLN__softmax_full_mha__glu_gated_swiglu__prompt_kernel(
    A_x: jax.Array,
    A_wqkv: jax.Array,
    A_wo: jax.Array,
    B_x: jax.Array,
    B_w1: jax.Array,
    B_w3: jax.Array,
    B_w2: jax.Array,
):
    bm = 512
    bt = 512
    sq = 128
    fch = F_CHUNKS
    wt_where = 'loop'
    del B_x
    x = A_x.reshape(S, D)
    hbm = pl.BlockSpec(memory_space=pl.ANY)
    out = pl.pallas_call(
        _make_kernel(bm, bt, sq, fch, wt_where),
        grid=(S // bt,),
        in_specs=[hbm] * 6,
        out_specs=pl.BlockSpec((bt, D), lambda i: (i, 0)),
        out_shape=jax.ShapeDtypeStruct((S, D), A_x.dtype),
        scratch_shapes=[
            pltpu.VMEM((S, D), jnp.bfloat16),
            pltpu.VMEM((D, 3 * D), jnp.bfloat16),
            pltpu.VMEM((D, D), jnp.bfloat16),
            pltpu.VMEM((F, D), jnp.bfloat16),
            pltpu.VMEM((F, D), jnp.bfloat16),
            pltpu.VMEM((FP, D), jnp.bfloat16),
            pltpu.VMEM((3 * D, D), jnp.bfloat16),
            pltpu.VMEM((D, S), jnp.bfloat16),
            pltpu.VMEM((D, D), jnp.bfloat16),
            pltpu.VMEM((D, FP), jnp.bfloat16),
            pltpu.VMEM((NWIN, 128, S), jnp.float32),
            pltpu.VMEM((NWIN, S, 128), jnp.bfloat16),
            pltpu.VMEM((H, 32, S), jnp.bfloat16),
            pltpu.VMEM((D, S), jnp.float32),
            pltpu.VMEM((8 * NWIN, S), jnp.float32),
            pltpu.SemaphoreType.DMA((S // bm,)),
            pltpu.SemaphoreType.DMA((5,)),
        ],
        compiler_params=pltpu.CompilerParams(
            dimension_semantics=("arbitrary",), vmem_limit_bytes=110 * 1024 * 1024),
    )(x, A_wqkv, A_wo, B_w1.T, B_w3.T, B_w2)
    return out.reshape(A_x.shape)
```

```python
import math

import jax
import jax.numpy as jnp
import numpy as np
from jax import lax
from jax.experimental import pallas as pl
from jax.experimental.pallas import tpu as pltpu

S = 2048
D = 640
H = 32
DH = D // H
F = 1728
FP = 1792
HPW = 6
NWIN = 6
WSTRIDE = HPW * DH
NRED = 8 * H
EPS = 1e-5
QK_SCALE = DH ** -0.5 * math.log2(math.e)

SHIFT = 40.0
BOUND_MARGIN = 1.0 + 2.0 ** -6
L_MIN = 2.0 ** -60
L_MAX = 2.0 ** 52
F32_MAX = float(np.finfo(np.float32).max)

BM = 512
BT = 512
SQ = 512
F_CHUNKS = ((0, 512), (512, 512), (1024, 512), (1536, 192))

_NT = (((1,), (1,)), ((), ()))


def _layernorm(x, axis):
    m = jnp.mean(x, axis=axis, keepdims=True)
    xc = x - m
    v = jnp.mean(xc * xc, axis=axis, keepdims=True)
    return xc * lax.rsqrt(v + EPS)


def _kernel(x_hbm, wqkv_hbm, wo_hbm, w1t_hbm, w3t_hbm, w2_hbm, out_ref,
            x_ref, wqkv_ref, wo_ref, w1t_ref, w3t_ref, w2_ref,
            wt_ref, xt_ref, wot_ref, w2t_ref, qtw_ref, kw_ref, vt_ref, ot_ref, qn_ref,
            xsem, wsem, osem):
    step = pl.program_id(0)
    nrb = S // BM

    def head_acc(h, q0, nq, true_max):
        rows = lax.broadcasted_iota(jnp.int32, (128, nq), 0)
        c = h // HPW
        hl = h - c * HPW
        keep = (rows >= hl * DH) & (rows < hl * DH + DH)
        if not true_max:
            keep = keep | (rows == WSTRIDE + hl)
        qm = jnp.where(keep, qtw_ref[c, :, pl.ds(q0, nq)], 0.0).astype(jnp.bfloat16)
        s = jnp.dot(kw_ref[c], qm, preferred_element_type=jnp.float32)
        if true_max:
            s = s - jnp.max(s, axis=0, keepdims=True)
        p = jnp.exp2(s).astype(jnp.bfloat16)
        return jnp.dot(vt_ref[h], p, preferred_element_type=jnp.float32)

    def head_pair(p, q0, nq, true_max):
        row8 = lax.broadcasted_iota(jnp.int32, (8, nq), 0)
        ae = head_acc(2 * p, q0, nq, true_max)
        ao = head_acc(2 * p + 1, q0, nq, true_max)
        le, lo = ae[24:32], ao[24:32]
        re, ro = 1.0 / le, 1.0 / lo
        mid = jnp.where(row8 < 4, ae[16:24] * re, ao[0:8] * ro)
        blk = jnp.concatenate([ae[0:8] * re, ae[8:16] * re, mid, ao[8:16] * ro, ao[16:24] * ro], axis=0)
        ot_ref[pl.ds(pl.multiple_of(p * 2 * DH, 8), 2 * DH), pl.ds(q0, nq)] = blk
        good = jnp.where((jnp.minimum(le, lo) >= L_MIN) & (jnp.maximum(le, lo) <= L_MAX), 1.0, 0.0)
        finite = jnp.where(jnp.abs(blk) <= F32_MAX, 1.0, 0.0)
        for g in range(2 * DH // 8):
            good = jnp.minimum(good, finite[8 * g:8 * g + 8])
        return good

    def x_copy(i):
        return pltpu.make_async_copy(x_hbm.at[pl.ds(i * BM, BM)], x_ref.at[pl.ds(i * BM, BM)], xsem.at[i])

    @pl.when(step == 0)
    def _project_and_attend():
        wcopies = [pltpu.make_async_copy(wqkv_hbm.at[:, pl.ds(c * D, D)], wqkv_ref.at[c], wsem.at[c])
                   for c in range(3)]
        ocopies = [
            pltpu.make_async_copy(wo_hbm, wo_ref, osem.at[0]),
            pltpu.make_async_copy(w2_hbm, w2_ref.at[pl.ds(0, F)], osem.at[1]),
            pltpu.make_async_copy(w1t_hbm, w1t_ref, osem.at[2]),
            pltpu.make_async_copy(w3t_hbm, w3t_ref, osem.at[3]),
        ]
        w2_ref[F:FP, :] = jnp.zeros((FP - F, D), jnp.bfloat16)
        for cp in wcopies:
            cp.start()
        x_copy(0).start()
        for c in range(3):
            wcopies[c].wait()
            if c == 0:
                for i in range(1, nrb):
                    x_copy(i).start()
                for cp in ocopies:
                    cp.start()
            wt_ref[c * D:(c + 1) * D, :] = wqkv_ref[c].astype(jnp.float32).T.astype(jnp.bfloat16)

        r = lax.broadcasted_iota(jnp.int32, (8 * NWIN, NRED), 0)
        f = lax.broadcasted_iota(jnp.int32, (8 * NWIN, NRED), 1)
        head = (r // 8) * HPW + (r % 8)
        sel = jnp.where(((r % 8) < HPW) & (f // 8 == head), 1.0, 0.0).astype(jnp.bfloat16)
        row8 = lax.broadcasted_iota(jnp.int32, (H // 2, 8, BM), 1)
        wrow = lax.broadcasted_iota(jnp.int32, (128, BM), 0)

        def head_sq_norms(t):
            t2 = (t * t).reshape(H // 2, 2 * DH, BM)
            mid = t2[:, 16:24]
            even = t2[:, 0:8] + t2[:, 8:16] + jnp.where(row8 < 4, mid, 0.0)
            odd = t2[:, 24:32] + t2[:, 32:40] + jnp.where(row8 < 4, 0.0, mid)
            folded = jnp.concatenate([even, odd], axis=1).reshape(NRED, BM)
            return jnp.dot(sel, folded.astype(jnp.bfloat16), preferred_element_type=jnp.float32)

        def project_block(rb, kmax):
            r0 = pl.multiple_of(rb * BM, BM)
            x_copy(rb).wait()
            xb = x_ref[pl.ds(r0, BM), :]
            xt_ref[:, pl.ds(r0, BM)] = xb.T
            xh = _layernorm(xb.astype(jnp.float32), -1).astype(jnp.bfloat16)
            qkvt = lax.dot_general(wt_ref[...], xh, _NT, preferred_element_type=jnp.float32)
            q = (qkvt[0:D] * QK_SCALE).astype(jnp.bfloat16).astype(jnp.float32)
            k = qkvt[D:2 * D].astype(jnp.bfloat16).astype(jnp.float32)
            v = qkvt[2 * D:3 * D]
            qn_ref[:, pl.ds(r0, BM)] = head_sq_norms(q)
            kn = head_sq_norms(k)
            zpad = jnp.zeros((128, BM), jnp.float32)
            qp = jnp.concatenate([q, zpad], axis=0)
            kp = jnp.concatenate([k, zpad], axis=0)
            for c in range(NWIN):
                lo = c * WSTRIDE
                qtw_ref[c, 0:WSTRIDE, pl.ds(r0, BM)] = qp[lo:lo + WSTRIDE]
                kwin = jnp.where(wrow < WSTRIDE, kp[lo:lo + 128], 1.0)
                kw_ref[c, pl.ds(r0, BM), :] = kwin.T.astype(jnp.bfloat16)
            ones = jnp.ones((8, BM), jnp.float32)
            for h in range(H):
                a = (h * DH) // 8 * 8
                vt_ref[h, :, pl.ds(r0, BM)] = jnp.concatenate([v[a:a + 24], ones], axis=0).astype(jnp.bfloat16)
            return jnp.maximum(kmax, kn)

        kmax = lax.fori_loop(0, nrb, project_block, jnp.zeros((8 * NWIN, BM), jnp.float32))
        kmax = jnp.max(kmax, axis=1, keepdims=True)
        shift = SHIFT - jnp.sqrt(qn_ref[...] * kmax) * BOUND_MARGIN
        for c in range(NWIN):
            qtw_ref[c, WSTRIDE:128, :] = shift[8 * c:8 * c + 8]

        for cp in ocopies:
            cp.wait()

        def attend_pair(p, good):
            g = head_pair(p, 0, S, False)
            f0 = pl.multiple_of(jnp.minimum(p, FP // 128 - 1) * 128, 128)
            w2t_ref[:, pl.ds(f0, 128)] = w2_ref[pl.ds(f0, 128), :].T
            o0 = pl.multiple_of(jnp.minimum(p, D // 128 - 1) * 128, 128)
            wot_ref[:, pl.ds(o0, 128)] = wo_ref[pl.ds(o0, 128), :].T
            return jnp.minimum(good, g)

        good = lax.fori_loop(0, H // 2, attend_pair, jnp.ones((8, S), jnp.float32))

        @pl.when(jnp.min(good) < 0.5)
        def _fallback():
            def body(i, carry):
                qb = i // (H // 2)
                head_pair(i - qb * (H // 2), pl.multiple_of(qb * SQ, SQ), SQ, True)
                return carry
            lax.fori_loop(0, (S // SQ) * (H // 2), body, 0)

    q0 = pl.multiple_of(step * BT, BT)
    o = ot_ref[:, pl.ds(q0, BT)].astype(jnp.bfloat16)
    h = xt_ref[:, pl.ds(q0, BT)].astype(jnp.float32) + jnp.dot(
        wot_ref[...], o, preferred_element_type=jnp.float32)
    hn = _layernorm(h, 0).astype(jnp.bfloat16)
    y = h
    for f0, fw in F_CHUNKS:
        g = jnp.dot(w1t_ref[f0:f0 + fw, :], hn, preferred_element_type=jnp.float32)
        u = jnp.dot(w3t_ref[f0:f0 + fw, :], hn, preferred_element_type=jnp.float32)
        a = (g * jax.nn.sigmoid(g) * u).astype(jnp.bfloat16)
        y = y + jnp.dot(w2t_ref[:, f0:f0 + fw], a, preferred_element_type=jnp.float32)
    out_ref[...] = y.astype(out_ref.dtype).T


@jax.jit
def pallas_sequential_preLN__softmax_full_mha__glu_gated_swiglu__prompt_kernel(
    A_x: jax.Array,
    A_wqkv: jax.Array,
    A_wo: jax.Array,
    B_x: jax.Array,
    B_w1: jax.Array,
    B_w3: jax.Array,
    B_w2: jax.Array,
):
    del B_x
    hbm = pl.BlockSpec(memory_space=pl.ANY)
    out = pl.pallas_call(
        _kernel,
        grid=(S // BT,),
        in_specs=[hbm] * 6,
        out_specs=pl.BlockSpec((BT, D), lambda i: (i, 0)),
        out_shape=jax.ShapeDtypeStruct((S, D), A_x.dtype),
        scratch_shapes=[
            pltpu.VMEM((S, D), jnp.bfloat16),
            pltpu.VMEM((3, D, D), jnp.bfloat16),
            pltpu.VMEM((D, D), jnp.bfloat16),
            pltpu.VMEM((F, D), jnp.bfloat16),
            pltpu.VMEM((F, D), jnp.bfloat16),
            pltpu.VMEM((FP, D), jnp.bfloat16),
            pltpu.VMEM((3 * D, D), jnp.bfloat16),
            pltpu.VMEM((D, S), jnp.bfloat16),
            pltpu.VMEM((D, D), jnp.bfloat16),
            pltpu.VMEM((D, FP), jnp.bfloat16),
            pltpu.VMEM((NWIN, 128, S), jnp.float32),
            pltpu.VMEM((NWIN, S, 128), jnp.bfloat16),
            pltpu.VMEM((H, 32, S), jnp.bfloat16),
            pltpu.VMEM((D, S), jnp.float32),
            pltpu.VMEM((8 * NWIN, S), jnp.float32),
            pltpu.SemaphoreType.DMA((S // BM,)),
            pltpu.SemaphoreType.DMA((3,)),
            pltpu.SemaphoreType.DMA((4,)),
        ],
        compiler_params=pltpu.CompilerParams(
            dimension_semantics=("arbitrary",), vmem_limit_bytes=110 * 1024 * 1024),
    )(A_x.reshape(S, D), A_wqkv, A_wo, B_w1.T, B_w3.T, B_w2)
    return out.reshape(A_x.shape)
```

```python
import math

import jax
import jax.numpy as jnp
import numpy as np
from jax import lax
from jax.experimental import pallas as pl
from jax.experimental.pallas import tpu as pltpu

S = 2048
D = 640
H = 32
DH = D // H
F = 1728
FP = 1792
HPW = 6
NWIN = 6
WSTRIDE = HPW * DH
NRED = 8 * H
EPS = 1e-5
QK_SCALE = DH ** -0.5 * math.log2(math.e)

SHIFT = 40.0
BOUND_MARGIN = 1.0 + 2.0 ** -6
L_MIN = 2.0 ** -60
L_MAX = 2.0 ** 52
F32_MAX = float(np.finfo(np.float32).max)

BM = 512
BT = 512
SQ = 512
F_CHUNKS = ((0, 512), (512, 512), (1024, 512), (1536, 192))

_NT = (((1,), (1,)), ((), ()))


def _layernorm(x, axis):
    m = jnp.mean(x, axis=axis, keepdims=True)
    xc = x - m
    v = jnp.mean(xc * xc, axis=axis, keepdims=True)
    return xc * lax.rsqrt(v + EPS)


def _kernel(x_hbm, wqkv_hbm, wo_hbm, w1t_hbm, w3t_hbm, w2_hbm, out_ref,
            x_ref, wqkv_ref, wo_ref, w1t_ref, w3t_ref, w2_ref,
            wt_ref, xt_ref, wot_ref, w2t_ref, qtw_ref, kw_ref, vt_ref, ot_ref, qn_ref, qm_ref,
            xsem, wsem, osem):
    step = pl.program_id(0)
    nrb = S // BM

    def masked_q(h, q0, nq, true_max):
        rows = lax.broadcasted_iota(jnp.int32, (128, nq), 0)
        c = h // HPW
        hl = h - c * HPW
        keep = (rows >= hl * DH) & (rows < hl * DH + DH)
        if not true_max:
            keep = keep | (rows == WSTRIDE + hl)
        return jnp.where(keep, qtw_ref[c, :, pl.ds(q0, nq)], 0.0).astype(jnp.bfloat16)

    def head_acc(h, q0, nq, true_max, slot=None):
        c = h // HPW
        if true_max:
            qm = masked_q(h, q0, nq, True)
        else:
            qm = qm_ref[slot]
        s = jnp.dot(kw_ref[c], qm, preferred_element_type=jnp.float32)
        if true_max:
            s = s - jnp.max(s, axis=0, keepdims=True)
        p = jnp.exp2(s).astype(jnp.bfloat16)
        return jnp.dot(vt_ref[h], p, preferred_element_type=jnp.float32)

    def head_pair(p, q0, nq, true_max):
        row8 = lax.broadcasted_iota(jnp.int32, (8, nq), 0)
        ae = head_acc(2 * p, q0, nq, true_max, 0)
        ao = head_acc(2 * p + 1, q0, nq, true_max, 1)
        le, lo = ae[24:32], ao[24:32]
        re, ro = 1.0 / le, 1.0 / lo
        mid = jnp.where(row8 < 4, ae[16:24] * re, ao[0:8] * ro)
        blk = jnp.concatenate([ae[0:8] * re, ae[8:16] * re, mid, ao[8:16] * ro, ao[16:24] * ro], axis=0)
        ot_ref[pl.ds(pl.multiple_of(p * 2 * DH, 8), 2 * DH), pl.ds(q0, nq)] = blk
        good = jnp.where((jnp.minimum(le, lo) >= L_MIN) & (jnp.maximum(le, lo) <= L_MAX), 1.0, 0.0)
        finite = jnp.where(jnp.abs(blk) <= F32_MAX, 1.0, 0.0)
        for g in range(2 * DH // 8):
            good = jnp.minimum(good, finite[8 * g:8 * g + 8])
        return good

    def x_copy(i):
        return pltpu.make_async_copy(x_hbm.at[pl.ds(i * BM, BM)], x_ref.at[pl.ds(i * BM, BM)], xsem.at[i])

    @pl.when(step == 0)
    def _project_and_attend():
        wcopies = [pltpu.make_async_copy(wqkv_hbm.at[:, pl.ds(c * D, D)], wqkv_ref.at[c], wsem.at[c])
                   for c in range(3)]
        ocopies = [
            pltpu.make_async_copy(wo_hbm, wo_ref, osem.at[0]),
            pltpu.make_async_copy(w2_hbm, w2_ref.at[pl.ds(0, F)], osem.at[1]),
            pltpu.make_async_copy(w1t_hbm, w1t_ref, osem.at[2]),
            pltpu.make_async_copy(w3t_hbm, w3t_ref, osem.at[3]),
        ]
        w2_ref[F:FP, :] = jnp.zeros((FP - F, D), jnp.bfloat16)
        for cp in wcopies:
            cp.start()
        x_copy(0).start()
        for c in range(3):
            wcopies[c].wait()
            if c == 0:
                for i in range(1, nrb):
                    x_copy(i).start()
                for cp in ocopies:
                    cp.start()
            wt_ref[c * D:(c + 1) * D, :] = wqkv_ref[c].astype(jnp.float32).T.astype(jnp.bfloat16)

        r = lax.broadcasted_iota(jnp.int32, (8 * NWIN, NRED), 0)
        f = lax.broadcasted_iota(jnp.int32, (8 * NWIN, NRED), 1)
        head = (r // 8) * HPW + (r % 8)
        sel = jnp.where(((r % 8) < HPW) & (f // 8 == head), 1.0, 0.0).astype(jnp.bfloat16)
        row8 = lax.broadcasted_iota(jnp.int32, (H // 2, 8, BM), 1)
        wrow = lax.broadcasted_iota(jnp.int32, (128, BM), 0)

        def head_sq_norms(t):
            t2 = (t * t).reshape(H // 2, 2 * DH, BM)
            mid = t2[:, 16:24]
            even = t2[:, 0:8] + t2[:, 8:16] + jnp.where(row8 < 4, mid, 0.0)
            odd = t2[:, 24:32] + t2[:, 32:40] + jnp.where(row8 < 4, 0.0, mid)
            folded = jnp.concatenate([even, odd], axis=1).reshape(NRED, BM)
            return jnp.dot(sel, folded.astype(jnp.bfloat16), preferred_element_type=jnp.float32)

        def project_block(rb, kmax):
            r0 = pl.multiple_of(rb * BM, BM)
            x_copy(rb).wait()
            xb = x_ref[pl.ds(r0, BM), :]
            xt_ref[:, pl.ds(r0, BM)] = xb.T
            xh = _layernorm(xb.astype(jnp.float32), -1).astype(jnp.bfloat16)
            qkvt = lax.dot_general(wt_ref[...], xh, _NT, preferred_element_type=jnp.float32)
            q = (qkvt[0:D] * QK_SCALE).astype(jnp.bfloat16).astype(jnp.float32)
            k = qkvt[D:2 * D].astype(jnp.bfloat16).astype(jnp.float32)
            v = qkvt[2 * D:3 * D]
            qn_ref[:, pl.ds(r0, BM)] = head_sq_norms(q)
            kn = head_sq_norms(k)
            zpad = jnp.zeros((128, BM), jnp.float32)
            qp = jnp.concatenate([q, zpad], axis=0)
            kp = jnp.concatenate([k, zpad], axis=0)
            for c in range(NWIN):
                lo = c * WSTRIDE
                qtw_ref[c, 0:WSTRIDE, pl.ds(r0, BM)] = qp[lo:lo + WSTRIDE]
                kwin = jnp.where(wrow < WSTRIDE, kp[lo:lo + 128], 1.0)
                kw_ref[c, pl.ds(r0, BM), :] = kwin.T.astype(jnp.bfloat16)
            ones = jnp.ones((8, BM), jnp.float32)
            for h in range(H):
                a = (h * DH) // 8 * 8
                vt_ref[h, :, pl.ds(r0, BM)] = jnp.concatenate([v[a:a + 24], ones], axis=0).astype(jnp.bfloat16)
            for t in range(BM // 128):
                kmax = jnp.maximum(kmax, kn[:, 128 * t:128 * (t + 1)])
            return kmax

        kmax = lax.fori_loop(0, nrb, project_block, jnp.zeros((8 * NWIN, 128), jnp.float32))
        kmax = jnp.max(kmax, axis=1, keepdims=True)
        shift = SHIFT - jnp.sqrt(qn_ref[...] * kmax) * BOUND_MARGIN
        for c in range(NWIN):
            qtw_ref[c, WSTRIDE:128, :] = shift[8 * c:8 * c + 8]

        for cp in ocopies:
            cp.wait()

        qm_ref[0] = masked_q(0, 0, S, False)
        qm_ref[1] = masked_q(1, 0, S, False)

        def attend_pair(p, good):
            g = head_pair(p, 0, S, False)
            pn = jnp.minimum(p + 1, H // 2 - 1)
            qm_ref[0] = masked_q(2 * pn, 0, S, False)
            qm_ref[1] = masked_q(2 * pn + 1, 0, S, False)
            f0 = pl.multiple_of(jnp.minimum(p, FP // 128 - 1) * 128, 128)
            w2t_ref[:, pl.ds(f0, 128)] = w2_ref[pl.ds(f0, 128), :].T
            o0 = pl.multiple_of(jnp.minimum(p, D // 128 - 1) * 128, 128)
            wot_ref[:, pl.ds(o0, 128)] = wo_ref[pl.ds(o0, 128), :].T
            return jnp.minimum(good, g)

        good = lax.fori_loop(0, H // 2, attend_pair, jnp.ones((8, S), jnp.float32))

        @pl.when(jnp.min(good) < 0.5)
        def _fallback():
            def body(i, carry):
                qb = i // (H // 2)
                head_pair(i - qb * (H // 2), pl.multiple_of(qb * SQ, SQ), SQ, True)
                return carry
            lax.fori_loop(0, (S // SQ) * (H // 2), body, 0)

    q0 = pl.multiple_of(step * BT, BT)
    o = ot_ref[:, pl.ds(q0, BT)].astype(jnp.bfloat16)
    h = xt_ref[:, pl.ds(q0, BT)].astype(jnp.float32) + jnp.dot(
        wot_ref[...], o, preferred_element_type=jnp.float32)
    hn = _layernorm(h, 0).astype(jnp.bfloat16)
    y = h
    for f0, fw in F_CHUNKS:
        g = jnp.dot(w1t_ref[f0:f0 + fw, :], hn, preferred_element_type=jnp.float32)
        u = jnp.dot(w3t_ref[f0:f0 + fw, :], hn, preferred_element_type=jnp.float32)
        a = (g * jax.nn.sigmoid(g) * u).astype(jnp.bfloat16)
        y = y + jnp.dot(w2t_ref[:, f0:f0 + fw], a, preferred_element_type=jnp.float32)
    out_ref[...] = y.astype(out_ref.dtype).T


@jax.jit
def pallas_sequential_preLN__softmax_full_mha__glu_gated_swiglu__prompt_kernel(
    A_x: jax.Array,
    A_wqkv: jax.Array,
    A_wo: jax.Array,
    B_x: jax.Array,
    B_w1: jax.Array,
    B_w3: jax.Array,
    B_w2: jax.Array,
):
    del B_x
    hbm = pl.BlockSpec(memory_space=pl.ANY)
    out = pl.pallas_call(
        _kernel,
        grid=(S // BT,),
        in_specs=[hbm] * 6,
        out_specs=pl.BlockSpec((BT, D), lambda i: (i, 0)),
        out_shape=jax.ShapeDtypeStruct((S, D), A_x.dtype),
        scratch_shapes=[
            pltpu.VMEM((S, D), jnp.bfloat16),
            pltpu.VMEM((3, D, D), jnp.bfloat16),
            pltpu.VMEM((D, D), jnp.bfloat16),
            pltpu.VMEM((F, D), jnp.bfloat16),
            pltpu.VMEM((F, D), jnp.bfloat16),
            pltpu.VMEM((FP, D), jnp.bfloat16),
            pltpu.VMEM((3 * D, D), jnp.bfloat16),
            pltpu.VMEM((D, S), jnp.bfloat16),
            pltpu.VMEM((D, D), jnp.bfloat16),
            pltpu.VMEM((D, FP), jnp.bfloat16),
            pltpu.VMEM((NWIN, 128, S), jnp.float32),
            pltpu.VMEM((NWIN, S, 128), jnp.bfloat16),
            pltpu.VMEM((H, 32, S), jnp.bfloat16),
            pltpu.VMEM((D, S), jnp.float32),
            pltpu.VMEM((8 * NWIN, S), jnp.float32),
            pltpu.VMEM((2, 128, S), jnp.bfloat16),
            pltpu.SemaphoreType.DMA((S // BM,)),
            pltpu.SemaphoreType.DMA((3,)),
            pltpu.SemaphoreType.DMA((4,)),
        ],
        compiler_params=pltpu.CompilerParams(
            dimension_semantics=("arbitrary",), vmem_limit_bytes=110 * 1024 * 1024),
    )(A_x.reshape(S, D), A_wqkv, A_wo, B_w1.T, B_w3.T, B_w2)
    return out.reshape(A_x.shape)
```

```python
import math

import jax
import jax.numpy as jnp
import numpy as np
from jax import lax
from jax.experimental import pallas as pl
from jax.experimental.pallas import tpu as pltpu

S = 2048
D = 640
H = 32
DH = D // H
F = 1728
FP = 1792
HPW = 6
NWIN = 6
WSTRIDE = HPW * DH
NRED = 8 * H
EPS = 1e-5
QK_SCALE = DH ** -0.5 * math.log2(math.e)

SHIFT = 40.0
BOUND_MARGIN = 1.0 + 2.0 ** -6
L_MIN = 2.0 ** -60
L_MAX = 2.0 ** 52
F32_MAX = float(np.finfo(np.float32).max)

BM = 512
BT = 512
SQ = 512

_NT = (((1,), (1,)), ((), ()))


def _layernorm(x, axis):
    m = jnp.mean(x, axis=axis, keepdims=True)
    xc = x - m
    v = jnp.mean(xc * xc, axis=axis, keepdims=True)
    return xc * lax.rsqrt(v + EPS)


def _kernel(x_hbm, wqkv_hbm, wo_hbm, w1t_hbm, w3t_hbm, w2_hbm, out_ref,
            x_ref, wqkv_ref, wo_ref, w1t_ref, w3t_ref, w2_ref,
            wt_ref, xt_ref, wot_ref, w2t_ref, qtw_ref, kw_ref, vt_ref, ot_ref, qn_ref, qm_ref,
            xsem, wsem, osem):
    step = pl.program_id(0)
    nrb = S // BM

    def masked_q(h, q0, nq, true_max):
        rows = lax.broadcasted_iota(jnp.int32, (128, nq), 0)
        c = h // HPW
        hl = h - c * HPW
        keep = (rows >= hl * DH) & (rows < hl * DH + DH)
        if not true_max:
            keep = keep | (rows == WSTRIDE + hl)
        return jnp.where(keep, qtw_ref[c, :, pl.ds(q0, nq)], 0.0).astype(jnp.bfloat16)

    def head_acc(h, q0, nq, true_max, slot=None):
        c = h // HPW
        qm = masked_q(h, q0, nq, True) if true_max else qm_ref[slot]
        s = jnp.dot(kw_ref[c], qm, preferred_element_type=jnp.float32)
        if true_max:
            s = s - jnp.max(s, axis=0, keepdims=True)
        p = jnp.exp2(s).astype(jnp.bfloat16)
        return jnp.dot(vt_ref[h], p, preferred_element_type=jnp.float32)

    def head_pair(p, q0, nq, true_max):
        row8 = lax.broadcasted_iota(jnp.int32, (8, nq), 0)
        ae = head_acc(2 * p, q0, nq, true_max, 0)
        ao = head_acc(2 * p + 1, q0, nq, true_max, 1)
        le, lo = ae[24:32], ao[24:32]
        re, ro = 1.0 / le, 1.0 / lo
        mid = jnp.where(row8 < 4, ae[16:24] * re, ao[0:8] * ro)
        blk = jnp.concatenate([ae[0:8] * re, ae[8:16] * re, mid, ao[8:16] * ro, ao[16:24] * ro], axis=0)
        ot_ref[pl.ds(pl.multiple_of(p * 2 * DH, 8), 2 * DH), pl.ds(q0, nq)] = blk
        good = jnp.where((jnp.minimum(le, lo) >= L_MIN) & (jnp.maximum(le, lo) <= L_MAX), 1.0, 0.0)
        finite = jnp.where(jnp.abs(blk) <= F32_MAX, 1.0, 0.0)
        for g in range(2 * DH // 8):
            good = jnp.minimum(good, finite[8 * g:8 * g + 8])
        return good

    def x_copy(i):
        return pltpu.make_async_copy(x_hbm.at[pl.ds(i * BM, BM)], x_ref.at[pl.ds(i * BM, BM)], xsem.at[i])

    @pl.when(step == 0)
    def _project_and_attend():
        wcopies = [pltpu.make_async_copy(wqkv_hbm.at[:, pl.ds(c * D, D)], wqkv_ref.at[c], wsem.at[c])
                   for c in range(3)]
        ocopies = [
            pltpu.make_async_copy(wo_hbm, wo_ref, osem.at[0]),
            pltpu.make_async_copy(w2_hbm, w2_ref.at[pl.ds(0, F)], osem.at[1]),
            pltpu.make_async_copy(w1t_hbm, w1t_ref, osem.at[2]),
            pltpu.make_async_copy(w3t_hbm, w3t_ref, osem.at[3]),
        ]
        w2_ref[F:FP, :] = jnp.zeros((FP - F, D), jnp.bfloat16)
        for cp in wcopies:
            cp.start()
        x_copy(0).start()
        for c in range(3):
            wcopies[c].wait()
            if c == 0:
                for i in range(1, nrb):
                    x_copy(i).start()
                for cp in ocopies:
                    cp.start()
            wt_ref[c * D:(c + 1) * D, :] = wqkv_ref[c].astype(jnp.float32).T.astype(jnp.bfloat16)

        r = lax.broadcasted_iota(jnp.int32, (8 * NWIN, NRED), 0)
        f = lax.broadcasted_iota(jnp.int32, (8 * NWIN, NRED), 1)
        head = (r // 8) * HPW + (r % 8)
        sel = jnp.where(((r % 8) < HPW) & (f // 8 == head), 1.0, 0.0).astype(jnp.bfloat16)
        row8 = lax.broadcasted_iota(jnp.int32, (H // 2, 8, BM), 1)
        wrow = lax.broadcasted_iota(jnp.int32, (128, BM), 0)

        def head_sq_norms(t):
            t2 = (t * t).reshape(H // 2, 2 * DH, BM)
            mid = t2[:, 16:24]
            even = t2[:, 0:8] + t2[:, 8:16] + jnp.where(row8 < 4, mid, 0.0)
            odd = t2[:, 24:32] + t2[:, 32:40] + jnp.where(row8 < 4, 0.0, mid)
            folded = jnp.concatenate([even, odd], axis=1).reshape(NRED, BM)
            return jnp.dot(sel, folded.astype(jnp.bfloat16), preferred_element_type=jnp.float32)

        def project_block(rb, kmax):
            r0 = pl.multiple_of(rb * BM, BM)
            x_copy(rb).wait()
            xb = x_ref[pl.ds(r0, BM), :]
            xt_ref[:, pl.ds(r0, BM)] = xb.T
            xh = _layernorm(xb.astype(jnp.float32), -1).astype(jnp.bfloat16)
            qkvt = lax.dot_general(wt_ref[...], xh, _NT, preferred_element_type=jnp.float32)
            q = (qkvt[0:D] * QK_SCALE).astype(jnp.bfloat16).astype(jnp.float32)
            k = qkvt[D:2 * D].astype(jnp.bfloat16).astype(jnp.float32)
            v = qkvt[2 * D:3 * D]
            qn_ref[:, pl.ds(r0, BM)] = head_sq_norms(q)
            kn = head_sq_norms(k)
            zpad = jnp.zeros((128, BM), jnp.float32)
            qp = jnp.concatenate([q, zpad], axis=0)
            kp = jnp.concatenate([k, zpad], axis=0)
            for c in range(NWIN):
                lo = c * WSTRIDE
                qtw_ref[c, 0:WSTRIDE, pl.ds(r0, BM)] = qp[lo:lo + WSTRIDE]
                kwin = jnp.where(wrow < WSTRIDE, kp[lo:lo + 128], 1.0)
                kw_ref[c, pl.ds(r0, BM), :] = kwin.T.astype(jnp.bfloat16)
            ones = jnp.ones((8, BM), jnp.float32)
            for h in range(H):
                a = (h * DH) // 8 * 8
                vt_ref[h, :, pl.ds(r0, BM)] = jnp.concatenate([v[a:a + 24], ones], axis=0).astype(jnp.bfloat16)
            for t in range(BM // 128):
                kmax = jnp.maximum(kmax, kn[:, 128 * t:128 * (t + 1)])
            return kmax

        kmax = lax.fori_loop(0, nrb, project_block, jnp.zeros((8 * NWIN, 128), jnp.float32))
        kmax = jnp.max(kmax, axis=1, keepdims=True)
        shift = SHIFT - jnp.sqrt(qn_ref[...] * kmax) * BOUND_MARGIN
        for c in range(NWIN):
            qtw_ref[c, WSTRIDE:128, :] = shift[8 * c:8 * c + 8]

        for cp in ocopies:
            cp.wait()

        qm_ref[0] = masked_q(0, 0, S, False)
        qm_ref[1] = masked_q(1, 0, S, False)

        def attend_pair(p, good):
            g = head_pair(p, 0, S, False)
            pn = jnp.minimum(p + 1, H // 2 - 1)
            qm_ref[0] = masked_q(2 * pn, 0, S, False)
            qm_ref[1] = masked_q(2 * pn + 1, 0, S, False)
            f0 = pl.multiple_of(jnp.minimum(p, FP // 128 - 1) * 128, 128)
            w2t_ref[:, pl.ds(f0, 128)] = w2_ref[pl.ds(f0, 128), :].T
            o0 = pl.multiple_of(jnp.minimum(p, D // 128 - 1) * 128, 128)
            wot_ref[:, pl.ds(o0, 128)] = wo_ref[pl.ds(o0, 128), :].T
            return jnp.minimum(good, g)

        good = lax.fori_loop(0, H // 2, attend_pair, jnp.ones((8, S), jnp.float32))

        @pl.when(jnp.min(good) < 0.5)
        def _fallback():
            def body(i, carry):
                qb = i // (H // 2)
                head_pair(i - qb * (H // 2), pl.multiple_of(qb * SQ, SQ), SQ, True)
                return carry
            lax.fori_loop(0, (S // SQ) * (H // 2), body, 0)

    q0 = pl.multiple_of(step * BT, BT)
    o = ot_ref[:, pl.ds(q0, BT)].astype(jnp.bfloat16)
    h = xt_ref[:, pl.ds(q0, BT)].astype(jnp.float32) + jnp.dot(
        wot_ref[...], o, preferred_element_type=jnp.float32)
    hn = _layernorm(h, 0).astype(jnp.bfloat16)
    g = jnp.dot(w1t_ref[...], hn, preferred_element_type=jnp.float32)
    u = jnp.dot(w3t_ref[...], hn, preferred_element_type=jnp.float32)
    a = (g * jax.nn.sigmoid(g) * u).astype(jnp.bfloat16)
    y = h + jnp.dot(w2t_ref[:, 0:F], a, preferred_element_type=jnp.float32)
    out_ref[...] = y.T.astype(out_ref.dtype)


@jax.jit
def pallas_sequential_preLN__softmax_full_mha__glu_gated_swiglu__prompt_kernel(
    A_x: jax.Array,
    A_wqkv: jax.Array,
    A_wo: jax.Array,
    B_x: jax.Array,
    B_w1: jax.Array,
    B_w3: jax.Array,
    B_w2: jax.Array,
):
    del B_x
    hbm = pl.BlockSpec(memory_space=pl.ANY)
    out = pl.pallas_call(
        _kernel,
        grid=(S // BT,),
        in_specs=[hbm] * 6,
        out_specs=pl.BlockSpec((BT, D), lambda i: (i, 0)),
        out_shape=jax.ShapeDtypeStruct((S, D), A_x.dtype),
        scratch_shapes=[
            pltpu.VMEM((S, D), jnp.bfloat16),
            pltpu.VMEM((3, D, D), jnp.bfloat16),
            pltpu.VMEM((D, D), jnp.bfloat16),
            pltpu.VMEM((F, D), jnp.bfloat16),
            pltpu.VMEM((F, D), jnp.bfloat16),
            pltpu.VMEM((FP, D), jnp.bfloat16),
            pltpu.VMEM((3 * D, D), jnp.bfloat16),
            pltpu.VMEM((D, S), jnp.bfloat16),
            pltpu.VMEM((D, D), jnp.bfloat16),
            pltpu.VMEM((D, FP), jnp.bfloat16),
            pltpu.VMEM((NWIN, 128, S), jnp.float32),
            pltpu.VMEM((NWIN, S, 128), jnp.bfloat16),
            pltpu.VMEM((H, 32, S), jnp.bfloat16),
            pltpu.VMEM((D, S), jnp.float32),
            pltpu.VMEM((8 * NWIN, S), jnp.float32),
            pltpu.VMEM((2, 128, S), jnp.bfloat16),
            pltpu.SemaphoreType.DMA((S // BM,)),
            pltpu.SemaphoreType.DMA((3,)),
            pltpu.SemaphoreType.DMA((4,)),
        ],
        compiler_params=pltpu.CompilerParams(
            dimension_semantics=("arbitrary",), vmem_limit_bytes=110 * 1024 * 1024),
    )(A_x.reshape(S, D), A_wqkv, A_wo, B_w1.T, B_w3.T, B_w2)
    return out.reshape(A_x.shape)
```
